```python
import os as _os
_os.environ.setdefault("JAX_PLATFORMS", "cpu")
import jax
import jax.numpy as jnp

def _softmax(x, axis=-1):
    return jax.nn.softmax(x, axis=axis)
def _gelu(x):
    return jax.nn.gelu(x, approximate=True)
def _silu(x):
    return jax.nn.silu(x)
def _sigmoid(x):
    return jax.nn.sigmoid(x)
def _layernorm(x, axis=-1, eps=1e-5):
    m = jnp.mean(x, axis=axis, keepdims=True)
    v = jnp.var(x, axis=axis, keepdims=True)
    return (x - m) / jnp.sqrt(v + eps)
def _scatter_add(tgt, idx, src, axis=0):
    return tgt.at[idx].add(src)
def _segment_sum(src, seg, n):
    return jax.ops.segment_sum(src, seg, n)
class _Rng:
    def __init__(self, key):
        self._k = key
    def _next(self):
        self._k, sub = jax.random.split(self._k)
        return sub
    def normal(self, shape):
        return jax.random.normal(self._next(), shape, dtype=jnp.bfloat16)
    def randint(self, lo, hi, shape):
        return jax.random.randint(self._next(), shape, lo, hi, dtype=jnp.int32)
    def uniform(self, shape, lo=0.0, hi=1.0):
        return jax.random.uniform(self._next(), shape, jnp.bfloat16, lo, hi)
    def permutation(self, n):
        return jax.random.permutation(self._next(), n)


kernel_name = 'concat_heads__sliding_block_cached__sliding_block_cached__decode'

def setup_inputs():
    _rng = _Rng(jax.random.key(int.from_bytes(__import__("os").urandom(4), "little")))
    _w = (lambda a: (lambda t: t.astype(jnp.bfloat16) if jnp.issubdtype(t.dtype, jnp.floating) else t)(jnp.asarray(a)))
    def _A_setup():
        B, Sq, D = 4, 1, 576
        Hq, Hkv, Sk, Dh = 32, 16, 8192, 128
        assert Hq % Hkv == 0, (Hq, Hkv)
        return {
            "x": _w((lambda *s: _rng.normal(s) * 0.8)(B, Sq, D)),
            "k_cache": _w((lambda *s: _rng.normal(s) * 0.8)(B, Hkv, Sk, Dh)),
            "v_cache": _w((lambda *s: _rng.normal(s) * 0.05)(B, Hkv, Sk, Dh)),
            "wq": _w((lambda *s: _rng.normal(s) * 0.8)(D, Hq * Dh) * (D ** -0.5)),
            "wo": _w((lambda *s: _rng.normal(s) * 0.05)(Hq * Dh, D) * ((Hq * Dh) ** -0.5)),
        }
    _A_in = _A_setup()

    def _B_setup():
        B, Sq, D = 4, 1, 576
        Hq, Hkv, Sk, Dh = 32, 16, 8192, 128
        assert Hq % Hkv == 0, (Hq, Hkv)
        return {
            "x": _w((lambda *s: _rng.normal(s) * 0.8)(B, Sq, D)),
            "k_cache": _w((lambda *s: _rng.normal(s) * 0.8)(B, Hkv, Sk, Dh)),
            "v_cache": _w((lambda *s: _rng.normal(s) * 0.05)(B, Hkv, Sk, Dh)),
            "wq": _w((lambda *s: _rng.normal(s) * 0.8)(D, Hq * Dh) * (D ** -0.5)),
            "wo": _w((lambda *s: _rng.normal(s) * 0.05)(Hq * Dh, D) * ((Hq * Dh) ** -0.5)),
        }
    _B_in = _B_setup()

    return {
        "A_x": _A_in["x"],
        "A_k_cache": _A_in["k_cache"],
        "A_v_cache": _A_in["v_cache"],
        "A_wq": _A_in["wq"],
        "A_wo": _A_in["wo"],
        "B_x": _B_in["x"],
        "B_k_cache": _B_in["k_cache"],
        "B_v_cache": _B_in["v_cache"],
        "B_wq": _B_in["wq"],
        "B_wo": _B_in["wo"],
    }

def reference(A_x, A_k_cache, A_v_cache, A_wq, A_wo, B_x, B_k_cache, B_v_cache, B_wq, B_wo):
    def _A_ref(x, k_cache, v_cache, wq, wo):
        B, Sq, D = x.shape
        Hq, Dh = 32, 128
        Hkv, Sk = k_cache.shape[1], k_cache.shape[2]
        W = min(4096, max(256, Sk // 4))
        rep = Hq // Hkv
        q = (lambda x, *d: x.transpose(*d))((x @ wq).reshape(B, Sq, Hq, Dh), 0, 2, 1, 3)
        k = jnp.repeat(k_cache[:, :, Sk - W:, :], rep, axis=1)
        v = jnp.repeat(v_cache[:, :, Sk - W:, :], rep, axis=1)
        scores = jnp.einsum("bhqd,bhkd->bhqk", q, k) * (Dh ** -0.5)
        p = _softmax(scores, axis=-1)
        o = jnp.einsum("bhqk,bhkd->bhqd", p, v)
        return (lambda x, *d: x.transpose(*d))(o, 0, 2, 1, 3).reshape(B, Sq, Hq * Dh) @ wo

    def _B_ref(x, k_cache, v_cache, wq, wo):
        B, Sq, D = x.shape
        Hq, Dh = 32, 128
        Hkv, Sk = k_cache.shape[1], k_cache.shape[2]
        W = min(4096, max(256, Sk // 4))
        rep = Hq // Hkv
        q = (lambda x, *d: x.transpose(*d))((x @ wq).reshape(B, Sq, Hq, Dh), 0, 2, 1, 3)
        k = jnp.repeat(k_cache[:, :, Sk - W:, :], rep, axis=1)
        v = jnp.repeat(v_cache[:, :, Sk - W:, :], rep, axis=1)
        scores = jnp.einsum("bhqd,bhkd->bhqk", q, k) * (Dh ** -0.5)
        p = _softmax(scores, axis=-1)
        o = jnp.einsum("bhqk,bhkd->bhqd", p, v)
        return (lambda x, *d: x.transpose(*d))(o, 0, 2, 1, 3).reshape(B, Sq, Hq * Dh) @ wo

    a = _A_ref(A_x, A_k_cache, A_v_cache, A_wq, A_wo)
    b = _B_ref(B_x, B_k_cache, B_v_cache, B_wq, B_wo)
    return jnp.concatenate([a, b], axis=-1)
```

```python
import jax
import jax.numpy as jnp
from jax import lax
import jax.experimental.pallas as pl
import jax.experimental.pallas.tpu as pltpu

_NT = (((1,), (1,)), ((), ()))
_NN = (((1,), (0,)), ((), ()))


@jax.jit
def pallas_concat_heads__sliding_block_cached__sliding_block_cached__decode_kernel(
    A_x: jax.Array,
    A_k_cache: jax.Array,
    A_v_cache: jax.Array,
    A_wq: jax.Array,
    A_wo: jax.Array,
    B_x: jax.Array,
    B_k_cache: jax.Array,
    B_v_cache: jax.Array,
    B_wq: jax.Array,
    B_wo: jax.Array,
):
    B, Sq, D = A_x.shape
    Hq, Dh = 32, 128
    Hkv, Sk = A_k_cache.shape[1], A_k_cache.shape[2]
    W = min(4096, max(256, Sk // 4))
    rep = Hq // Hkv
    assert (B, Sq, rep) == (4, 1, 2)
    S0 = Sk - W
    C = rep * Dh
    scale = Dh ** -0.5
    NG = 4

    def kernel(xa, ka, va, wqa, woa, xb, kb, vb, wqb, wob, o_ref,
               xbuf, kbuf, vbuf, wqbuf, wobuf, acc_ref, xsem, ksem, vsem, wqsem, wosem):
        probs = ((xa, ka, va, wqa, woa), (xb, kb, vb, wqb, wob))

        def copies(p, h, slot):
            _, k, v, wq, wo = probs[p]
            col = h * C if isinstance(h, int) else pl.multiple_of(h * C, C)
            cwq = pltpu.make_async_copy(wq.at[:, pl.ds(col, C)], wqbuf.at[slot], wqsem.at[slot])
            cwo = pltpu.make_async_copy(wo.at[:, pl.ds(col, C)], wobuf.at[slot], wosem.at[slot])
            ck = [pltpu.make_async_copy(k.at[b, h, pl.ds(S0, W), :], kbuf.at[slot, b], ksem.at[slot, b])
                  for b in range(B)]
            cv = [pltpu.make_async_copy(v.at[b, h, pl.ds(S0, W), :], vbuf.at[slot, b], vsem.at[slot, b])
                  for b in range(B)]
            return cwq, ck, cv, cwo

        def start_group(p, h, slot):
            cwq, ck, cv, cwo = copies(p, h, slot)
            cwq.start(priority=0)
            cwo.start(priority=1)
            for b in range(B):
                ck[b].start(priority=b % 2)
            for b in range(B):
                cv[b].start(priority=b % 2)

        xc = [pltpu.make_async_copy(probs[p][0], xbuf.at[p], xsem.at[p]) for p in range(2)]
        for p in range(2):
            xc[p].start()
        for g in range(NG):
            start_group(0, g, g)
        for p in range(2):
            xc[p].wait()

        row = lax.broadcasted_iota(jnp.int32, (8, Dh), 0)
        rowb = row % 4
        lo = row < 4
        rowb_w = lax.broadcasted_iota(jnp.int32, (8, W), 0) % 4

        for p in range(2):
            x4 = xbuf[p].astype(jnp.float32)
            x8 = jnp.concatenate([x4, x4], axis=0).astype(jnp.bfloat16)
            acc_ref[...] = jnp.zeros_like(acc_ref)

            def body(h, _, p=p, x8=x8):
                slot = (p * Hkv + h) % NG
                cwq, ck, cv, cwo = copies(p, h, slot)
                cwq.wait()
                qf = lax.dot_general(x8, wqbuf[slot], _NN, preferred_element_type=jnp.float32)
                q = jnp.where(lo, qf[:, :Dh], qf[:, Dh:]).astype(jnp.bfloat16)
                s = None
                for b in range(B):
                    ck[b].wait()
                    sb = lax.dot_general(q, kbuf[slot, b], _NT, preferred_element_type=jnp.float32)
                    s = sb if s is None else jnp.where(rowb_w == b, sb, s)
                s = s * scale
                m = jnp.max(s, axis=-1, keepdims=True)
                e = jnp.exp(s - m)
                l = jnp.sum(e, axis=-1, keepdims=True)
                pb = e.astype(jnp.bfloat16)
                o = None
                for b in range(B):
                    cv[b].wait()
                    ob = lax.dot_general(pb, vbuf[slot, b], _NN, preferred_element_type=jnp.float32)
                    o = ob if o is None else jnp.where(rowb == b, ob, o)
                cwo.wait()
                o = o / l
                z = jnp.concatenate([jnp.where(lo, o, 0.0), jnp.where(lo, 0.0, o)], axis=1).astype(jnp.bfloat16)
                acc_ref[...] += lax.dot_general(z, wobuf[slot], _NT, preferred_element_type=jnp.float32)
                hn = h + NG

                @pl.when(hn < Hkv)
                def _():
                    start_group(p, hn, slot)

                if p == 0:
                    @pl.when(hn >= Hkv)
                    def _():
                        start_group(1, hn - Hkv, slot)
                return 0

            lax.fori_loop(0, Hkv, body, 0)
            a = acc_ref[...]
            o_ref[:, p * D:(p + 1) * D] = (a[0:4] + a[4:8]).astype(o_ref.dtype)

    any_spec = pl.BlockSpec(memory_space=pl.ANY)
    out = pl.pallas_call(
        kernel,
        out_shape=jax.ShapeDtypeStruct((B, 2 * D), jnp.bfloat16),
        in_specs=[any_spec] * 10,
        out_specs=pl.BlockSpec(memory_space=pltpu.VMEM),
        scratch_shapes=[
            pltpu.VMEM((2, B, D), jnp.bfloat16),
            pltpu.VMEM((NG, B, W, Dh), jnp.bfloat16),
            pltpu.VMEM((NG, B, W, Dh), jnp.bfloat16),
            pltpu.VMEM((NG, D, C), jnp.bfloat16),
            pltpu.VMEM((NG, D, C), jnp.bfloat16),
            pltpu.VMEM((8, D), jnp.float32),
            pltpu.SemaphoreType.DMA((2,)),
            pltpu.SemaphoreType.DMA((NG, B)),
            pltpu.SemaphoreType.DMA((NG, B)),
            pltpu.SemaphoreType.DMA((NG,)),
            pltpu.SemaphoreType.DMA((NG,)),
        ],
        compiler_params=pltpu.CompilerParams(vmem_limit_bytes=100 * 1024 * 1024),
    )(A_x.reshape(B, D), A_k_cache, A_v_cache, A_wq, A_wo.T,
      B_x.reshape(B, D), B_k_cache, B_v_cache, B_wq, B_wo.T)
    return out.reshape(B, Sq, 2 * D)
```

```python
import functools

import jax
import jax.numpy as jnp
from jax import lax
import jax.experimental.pallas as pl
import jax.experimental.pallas.tpu as pltpu

_NT = (((1,), (1,)), ((), ()))
_NN = (((1,), (0,)), ((), ()))

_NCH = 11
_LAG0 = 30
_LAG1 = 90
_GAP = 2
_WRB = 8
_WSPLIT = 2


def _split_rows(total, n, q=16):
    units = total // q
    base, rem = divmod(units, n)
    sizes = [(base + 1) * q] * rem + [base * q] * (n - rem)
    offs = [sum(sizes[:i]) for i in range(n)]
    return list(zip(offs, sizes))


def _build_schedule(B):
    stream = []
    ready = {}
    for p in range(2):
        for b in range(B):
            for c in range(_NCH):
                stream.append((p, B + b, c, 1))
                stream.append((p, b, c, 0))
            ready[(p, b)] = len(stream) + _LAG0
            ready[(p, B + b)] = len(stream) + _LAG1
    ns = len(stream)
    pieces = []
    for p in range(2):
        chain = [("qproj", (), ready[(p, 0)] - _GAP)]
        chain += [("qk", (b,), ready[(p, b)]) for b in range(B)]
        chain += [("softmax", (), 0)]
        chain += [("pv", (b,), ready[(p, B + b)]) for b in range(B)]
        chain += [("oproj", (), 0)]
        last = -(10 ** 9)
        for name, args, pos in chain:
            pos = max(pos, last + _GAP)
            last = pos
            pieces.append((pos, p, name, args))
    pieces.sort(key=lambda t: (t[0], t[1]))
    assert max(t[0] for t in pieces) < 2 * ns
    first = {}
    for idx, (p, j, _, _) in enumerate(stream):
        first.setdefault((p, j), idx)
    for pos, p, name, args in pieces:
        if name in ("qk", "pv"):
            j = args[0] + (B if name == "pv" else 0)
            assert pos <= first[(p, j)] + ns
    return stream, pieces


@jax.jit
def pallas_concat_heads__sliding_block_cached__sliding_block_cached__decode_kernel(
    A_x: jax.Array,
    A_k_cache: jax.Array,
    A_v_cache: jax.Array,
    A_wq: jax.Array,
    A_wo: jax.Array,
    B_x: jax.Array,
    B_k_cache: jax.Array,
    B_v_cache: jax.Array,
    B_wq: jax.Array,
    B_wo: jax.Array,
):
    B, Sq, D = A_x.shape
    Hq, Dh = 32, 128
    Hkv, Sk = A_k_cache.shape[1], A_k_cache.shape[2]
    W = min(4096, max(256, Sk // 4))
    rep = Hq // Hkv
    assert (B, Sq, rep) == (4, 1, 2) and D % _WRB == 0
    R = B * rep
    S0 = Sk - W
    C = rep * Dh
    HD = Hq * Dh
    WC = HD // _WSPLIT
    scale = Dh ** -0.5
    chunks = _split_rows(W, _NCH)
    stream, pieces = _build_schedule(B)
    NS = len(stream)

    def kernel(xa, ka, va, wqa, woa, xb, kb, vb, wqb, wob, o_ref,
               xbuf, kvbuf, wbuf, acc_ref, q_ref, s_ref, p_ref, l_ref, oacc_ref,
               xsem, kvsem, wsem):
        probs = ((xa, ka, va, wqa, woa), (xb, kb, vb, wqb, wob))

        def start_chunk(h, idx):
            p, j, c, prio = stream[idx]
            off, sz = chunks[c]
            src = probs[p][1] if j < B else probs[p][2]
            pltpu.make_async_copy(
                src.at[j % B, h, pl.ds(S0 + off, sz), :],
                kvbuf.at[p, j, pl.ds(off, sz), :],
                kvsem.at[p, j],
            ).start(priority=prio)

        def wait_block(p, j):
            pltpu.make_async_copy(kvbuf.at[p, j], kvbuf.at[p, j], kvsem.at[p, j]).wait()

        def wait_weight(p, j):
            pltpu.make_async_copy(wbuf.at[p, j], wbuf.at[p, j], wsem.at[p, j]).wait()

        x_copies = [pltpu.make_async_copy(probs[p][0], xbuf.at[p], xsem.at[p]) for p in range(2)]

        def weight_rows(j, r, carry):
            r0 = pl.multiple_of(r * _WRB, _WRB)
            for cpiece in range(_WSPLIT):
                for p in (1, 0):
                    pltpu.make_async_copy(
                        probs[p][3 + j].at[pl.ds(r0, _WRB), pl.ds(cpiece * WC, WC)],
                        wbuf.at[p, j, pl.ds(r0, _WRB), pl.ds(cpiece * WC, WC)],
                        wsem.at[p, j],
                    ).start(priority=p)
            return carry

        lax.fori_loop(0, D // _WRB, functools.partial(weight_rows, 0), 0)
        for p in range(2):
            x_copies[p].start()
        lax.fori_loop(0, D // _WRB, functools.partial(weight_rows, 1), 0)

        row = lax.broadcasted_iota(jnp.int32, (R, Dh), 0)
        row_b = row % B
        lo = row < B
        row_b_w = lax.broadcasted_iota(jnp.int32, (R, W), 0) % B

        acc_ref[...] = jnp.zeros_like(acc_ref)
        for p in range(2):
            x_copies[p].wait()
            wait_weight(p, 0)

        def head_cols(h):
            return pl.ds(h * C if isinstance(h, int) else pl.multiple_of(h * C, C), C)

        def qproj(h, p):
            x4 = xbuf[p].astype(jnp.float32)
            x8 = jnp.concatenate([x4, x4], axis=0).astype(jnp.bfloat16)
            qf = lax.dot_general(x8, wbuf[p, 0, :, head_cols(h)], _NN,
                                 preferred_element_type=jnp.float32)
            q_ref[p] = jnp.where(lo, qf[:, :Dh], qf[:, Dh:])

        def qk(h, p, b):
            wait_block(p, b)
            q = q_ref[p].astype(jnp.bfloat16)
            sb = lax.dot_general(q, kvbuf[p, b], _NT, preferred_element_type=jnp.float32)
            if b == 0:
                s_ref[p] = sb
            else:
                s_ref[p] = jnp.where(row_b_w == b, sb, s_ref[p])

        def softmax(h, p):
            s = s_ref[p] * scale
            m = jnp.max(s, axis=-1, keepdims=True)
            e = jnp.exp(s - m)
            l_ref[p] = jnp.broadcast_to(jnp.sum(e, axis=-1, keepdims=True), (R, Dh))
            p_ref[p] = e

        def pv(h, p, b):
            wait_block(p, B + b)
            pb = p_ref[p].astype(jnp.bfloat16)
            ob = lax.dot_general(pb, kvbuf[p, B + b], _NN, preferred_element_type=jnp.float32)
            if b == 0:
                oacc_ref[p] = ob
            else:
                oacc_ref[p] = jnp.where(row_b == b, ob, oacc_ref[p])

        def oproj(h, p):
            if isinstance(h, int):
                if h == 0:
                    wait_weight(p, 1)
            else:
                pl.when(h == 0)(functools.partial(wait_weight, p, 1))
            o = oacc_ref[p] / l_ref[p]
            z = jnp.concatenate([jnp.where(lo, o, 0.0), jnp.where(lo, 0.0, o)], axis=1)
            acc_ref[p] += lax.dot_general(z.astype(jnp.bfloat16), wbuf[p, 1, :, head_cols(h)], _NT,
                                          preferred_element_type=jnp.float32)

        fns = dict(qproj=qproj, qk=qk, softmax=softmax, pv=pv, oproj=oproj)

        def body(h, carry):
            for idx in range(NS):
                start_chunk(h, idx)
                for pos, p, name, args in pieces:
                    if pos - NS == idx + 1:
                        pl.when(h > 0)(functools.partial(fns[name], h - 1, p, *args))
                    elif pos == idx + 1:
                        fns[name](h, p, *args)
            return carry

        lax.fori_loop(0, Hkv, body, 0)

        for pos, p, name, args in pieces:
            if pos > NS:
                fns[name](Hkv - 1, p, *args)
        for p in range(2):
            a = acc_ref[p]
            o_ref[:, p * D:(p + 1) * D] = (a[0:B] + a[B:R]).astype(o_ref.dtype)

    any_spec = pl.BlockSpec(memory_space=pl.ANY)
    out = pl.pallas_call(
        kernel,
        out_shape=jax.ShapeDtypeStruct((B, 2 * D), jnp.bfloat16),
        in_specs=[any_spec] * 10,
        out_specs=pl.BlockSpec(memory_space=pltpu.VMEM),
        scratch_shapes=[
            pltpu.VMEM((2, B, D), jnp.bfloat16),
            pltpu.VMEM((2, 2 * B, W, Dh), jnp.bfloat16),
            pltpu.VMEM((2, 2, D, HD), jnp.bfloat16),
            pltpu.VMEM((2, R, D), jnp.float32),
            pltpu.VMEM((2, R, Dh), jnp.float32),
            pltpu.VMEM((2, R, W), jnp.float32),
            pltpu.VMEM((2, R, W), jnp.float32),
            pltpu.VMEM((2, R, Dh), jnp.float32),
            pltpu.VMEM((2, R, Dh), jnp.float32),
            pltpu.SemaphoreType.DMA((2,)),
            pltpu.SemaphoreType.DMA((2, 2 * B)),
            pltpu.SemaphoreType.DMA((2, 2)),
        ],
        compiler_params=pltpu.CompilerParams(vmem_limit_bytes=100 * 1024 * 1024),
    )(A_x.reshape(B, D), A_k_cache, A_v_cache, A_wq, A_wo.T,
      B_x.reshape(B, D), B_k_cache, B_v_cache, B_wq, B_wo.T)
    return out.reshape(B, Sq, 2 * D)
```

```python
import functools

import jax
import jax.numpy as jnp
from jax import lax
import jax.experimental.pallas as pl
import jax.experimental.pallas.tpu as pltpu

_NT = (((1,), (1,)), ((), ()))
_NN = (((1,), (0,)), ((), ()))

_L = 4
_CR = 128
_LAG = 30
_VLAG = 64
_QPOS = 12
_OPOS = 76
_TAILC = 4
_WPARTS = 4
_WLATE = 4
_WPRE = 2
_OFFS = (-8, 16)


@jax.jit
def pallas_concat_heads__sliding_block_cached__sliding_block_cached__decode_kernel(
    A_x: jax.Array,
    A_k_cache: jax.Array,
    A_v_cache: jax.Array,
    A_wq: jax.Array,
    A_wo: jax.Array,
    B_x: jax.Array,
    B_k_cache: jax.Array,
    B_v_cache: jax.Array,
    B_wq: jax.Array,
    B_wo: jax.Array,
):
    B, Sq, D = A_x.shape
    Hq, Dh = 32, 128
    Hkv, Sk = A_k_cache.shape[1], A_k_cache.shape[2]
    W = min(4096, max(256, Sk // 4))
    rep = Hq // Hkv
    L, CR = _L, _CR
    S0 = Sk - W
    C = rep * Dh
    HD = Hq * Dh
    R = 8 * rep
    scale = Dh ** -0.5
    NCH = W // CR
    LP = L // 2
    N = (2 * B * Hkv) // L
    NHG = N // B
    ST = NCH // L
    SLOT = ST * 2 * L
    RBP = (D // 8) // _WPARTS
    WH = HD // 2
    assert (B, Sq, rep, NCH, L) == (4, 1, 2, 16, 4) and D == 8 * _WPARTS * RBP
    assert _LAG < SLOT and _VLAG == 2 * SLOT and NHG * LP == Hkv
    assert _WLATE * _WPARTS * 4 == L * NCH

    def lane_prob(j):
        return 1 - j // LP

    def head_of(hg, j):
        return hg + (j % LP) * NHG

    def rows_of(j, c):
        off = _OFFS[lane_prob(j)]
        lo = 0 if c == 0 else c * CR + off
        hi = W if c == NCH - 1 else (c + 1) * CR + off
        return lo, hi - lo

    def unit_info(n):
        return n % B, n // B, n % 2

    s0, s1 = [], []
    for s in range(ST * (L - 1)):
        for j in range(L):
            if s < ST * j:
                s1.append((1, j, N - 2, *rows_of(j, s), False))
                s0.append((0, j, N - 1, *rows_of(j, s), False))

    def v_last(j, cs, tail=False):
        return [(1, j, N - 1, *rows_of(j, c), tail) for c in cs]

    half = NCH // 2
    s0 += v_last(0, range(half))
    s0 += [e for pair in zip(v_last(0, range(half, NCH)), v_last(1, range(half, NCH))) for e in pair]
    s0 += v_last(1, range(half))
    s1 += v_last(2, range(NCH)) + v_last(3, range(NCH - _TAILC)) + v_last(3, range(NCH - _TAILC, NCH), True)
    assert len(s0) == len(s1)
    T0 = rows_of(L - 1, NCH - _TAILC)[0]
    TM = (T0 // CR) * CR

    def kernel(xa, ka, va, wqa, woa, xb, kb, vb, wqb, wob, o_ref,
               xbuf, kvbuf, wbuf, acc_ref, q_ref, p_ref, l_ref, oh_ref, otmp_ref,
               xsem, kvsem, wsem, tsem):
        probs = ((xa, ka, va, wqa, woa), (xb, kb, vb, wqb, wob))

        def rows_copy(info, j, kv, r0, nr, tail=False):
            b, hg, slot = info
            src = probs[lane_prob(j)][1 + kv]
            sem = tsem.at[0] if tail else kvsem.at[kv, j, slot]
            return pltpu.make_async_copy(
                src.at[b, head_of(hg, j), pl.ds(S0 + r0, nr), :],
                kvbuf.at[kv, j, slot, pl.ds(r0, nr), :],
                sem,
            )

        def wait_block(kv, j, slot):
            pltpu.make_async_copy(kvbuf.at[kv, j, slot], kvbuf.at[kv, j, slot], kvsem.at[kv, j, slot]).wait()

        def wait_weight(p, w):
            pltpu.make_async_copy(wbuf.at[p, w], wbuf.at[p, w], wsem.at[p, w]).wait()

        def w_copy(p, w, r, part, hf):
            r0 = (part * RBP + r) * 8
            if not isinstance(r0, int):
                r0 = pl.multiple_of(r0, 8)
            return pltpu.make_async_copy(
                probs[p][3 + w].at[pl.ds(r0, 8), pl.ds(hf * WH, WH)],
                wbuf.at[p, w, pl.ds(r0, 8), pl.ds(hf * WH, WH)],
                wsem.at[p, w],
            )

        x_copies = [pltpu.make_async_copy(probs[p][0], xbuf.at[p], xsem.at[p]) for p in range(2)]

        def weight_rows(w, r, carry):
            for hf in range(2):
                for part in range(_WPARTS):
                    for p in (1, 0):
                        w_copy(p, w, r, part, hf).start(priority=p)
            return carry

        n_mid = RBP - _WLATE - _WPRE
        for r in range(n_mid, n_mid + _WPRE):
            for hf in range(2):
                for p in (1, 0):
                    for part in range(_WPARTS):
                        w_copy(p, 1, r, part, hf).start(priority=1)
        lax.fori_loop(0, RBP, functools.partial(weight_rows, 0), 0)
        for p in range(2):
            x_copies[p].start()
        lax.fori_loop(0, n_mid, functools.partial(weight_rows, 1), 0)
        late_w = [(p, 1, r, part, hf) for p in (1, 0) for r in range(RBP - _WLATE, RBP)
                  for hf in range(2) for part in range(_WPARTS)]

        row_b = lax.broadcasted_iota(jnp.int32, (R, Dh), 0) % B
        acc_ref[...] = jnp.zeros_like(acc_ref)
        oh_ref[...] = jnp.zeros_like(oh_ref)

        def cols(h):
            return pl.ds(h * C if isinstance(h, int) else pl.multiple_of(h * C, C), C)

        def qproj(j, hg, par):
            p = lane_prob(j)
            x4 = xbuf[p].astype(jnp.float32)
            x8 = jnp.concatenate([x4, x4], axis=0).astype(jnp.bfloat16)
            qf = lax.dot_general(x8, wbuf[p, 0, :, cols(head_of(hg, j))], _NN,
                                 preferred_element_type=jnp.float32)
            q_ref[j, par] = jnp.concatenate([qf[:, :Dh], qf[:, Dh:]], axis=0).astype(jnp.bfloat16)

        def scores_softmax(j, info):
            _, hg, slot = info
            s = lax.dot_general(q_ref[j, hg % 2], kvbuf[0, j, slot], _NT,
                                preferred_element_type=jnp.float32) * scale
            m = jnp.max(s, axis=-1, keepdims=True)
            e = jnp.exp(s - m)
            l_ref[j, slot] = jnp.broadcast_to(jnp.sum(e, axis=-1, keepdims=True), (R, Dh))
            p_ref[j, slot] = e.astype(jnp.bfloat16)

        def pv_rows(j, info, r0, nr):
            slot = info[2]
            return lax.dot_general(p_ref[j, slot, :, pl.ds(r0, nr)], kvbuf[1, j, slot, pl.ds(r0, nr), :],
                                   _NN, preferred_element_type=jnp.float32)

        def pv_finish(j, info, o):
            b, hg, slot = info
            oh_ref[j, hg % 2] = jnp.where(row_b == b, o / l_ref[j, slot], oh_ref[j, hg % 2])

        def oproj(j, hg, valid=None):
            p = lane_prob(j)
            o = oh_ref[j, hg % 2]
            if valid is not None:
                o = jnp.where(valid, o, 0.0)
            z = jnp.concatenate([o[0:8], o[8:16]], axis=1).astype(jnp.bfloat16)
            acc_ref[p] += lax.dot_general(z, wbuf[p, 1, :, cols(head_of(hg, j))], _NT,
                                          preferred_element_type=jnp.float32)

        def write_out(p):
            o_ref[:, p * D:(p + 1) * D] = acc_ref[p, 0:B, :].astype(o_ref.dtype)

        def iteration(i):
            static = isinstance(i, int)
            infos = {d: unit_info(i - d) if (not static or i - d >= 0) else None for d in range(4)}
            actions = {}

            def consume(t):
                iq = infos[1]
                jv = (t - 2) % L
                iv = infos[2 if t >= 2 else 3]
                if iq is not None:
                    wait_block(0, t, iq[2])
                if iv is not None:
                    wait_block(1, jv, iv[2])
                if iq is not None:
                    scores_softmax(t, iq)
                if iv is not None:
                    pv_finish(jv, iv, pv_rows(jv, iv, 0, W))

            for t in range(L):
                actions[SLOT * t + _LAG] = functools.partial(consume, t)
            hgq = (i - 1) // L + 1
            if static:
                if i >= 1:
                    actions[_QPOS] = functools.partial(qproj, (i - 1) % L, hgq, hgq % 2)
            else:
                actions[_QPOS] = functools.partial(qproj, (i - 1) % L, jnp.minimum(hgq, NHG - 1), hgq % 2)
                io = jnp.maximum(i - 6, 0)
                actions[_OPOS] = functools.partial(oproj, io % L, io // L, i >= 6)
            idx = 0
            for s in range(NCH):
                for j in range(L):
                    dk = 0 if s >= ST * j else 1
                    ik, iv = infos[dk], infos[dk + 1]
                    if idx in actions:
                        actions[idx]()
                    if iv is not None:
                        rows_copy(iv, j, 1, *rows_of(j, s)).start(priority=1)
                    elif ik is not None:
                        w_copy(*late_w.pop(0)).start(priority=1)
                    if ik is not None:
                        rows_copy(ik, j, 0, *rows_of(j, s)).start(priority=0)
                    idx += 2

        iteration(0)
        for p in range(2):
            x_copies[p].wait()
            wait_weight(p, 0)
        for j in range(L):
            qproj(j, 0, 0)
        iteration(1)
        assert not late_w
        iteration(2)
        for p in range(2):
            wait_weight(p, 1)

        def body(i, carry):
            iteration(i)
            return carry

        lax.fori_loop(3, N, body, 0)

        ready = {(1, 2, N - 3): _LAG, (1, 3, N - 3): _LAG + SLOT}
        for t in range(L):
            ready[(0, t, N - 1)] = _LAG
            ready[(1, t, N - 2)] = _LAG + _VLAG
        for x, e in enumerate(s0):
            ready[e[:3]] = max(ready.get(e[:3], 0), 2 * (x + 1) + _LAG)
        for x, e in enumerate(s1):
            ready[e[:3]] = max(ready.get(e[:3], 0), 2 * (x + 1) + _LAG + _VLAG)

        def end_k(j, n):
            info = unit_info(n)
            wait_block(0, j, info[2])
            scores_softmax(j, info)

        def end_v(j, n):
            info = unit_info(n)
            if (j, n) != (L - 1, N - 1):
                wait_block(1, j, info[2])
                pv_finish(j, info, pv_rows(j, info, 0, W))
            else:
                rows_copy(info, j, 1, 0, T0).wait()
                otmp_ref[...] = pv_rows(j, info, 0, TM)
                rows_copy(info, j, 1, T0, W - T0, tail=True).wait()
                pv_finish(j, info, otmp_ref[...] + pv_rows(j, info, TM, W - TM))
            if n == N - 1:
                oproj(j, NHG - 1)
                if j % LP == LP - 1:
                    write_out(lane_prob(j))

        events = [(pos, kv, n, j, functools.partial(end_v if kv else end_k, j, n))
                  for (kv, j, n), pos in ready.items()]
        events.append((4, 2, 0, 0, functools.partial(oproj, 2, NHG - 2)))
        events.append((16, 2, 0, 0, functools.partial(oproj, 3, NHG - 2)))
        events.sort(key=lambda e: e[:4])
        for x in range(len(s0)):
            while events and events[0][0] <= 2 * x:
                events.pop(0)[4]()
            for prio, (kv, j, n, r0, nr, tail) in ((1, s1[x]), (0, s0[x])):
                rows_copy(unit_info(n), j, kv, r0, nr, tail=tail).start(priority=prio)
        for e in events:
            e[4]()

    any_spec = pl.BlockSpec(memory_space=pl.ANY)
    out = pl.pallas_call(
        kernel,
        out_shape=jax.ShapeDtypeStruct((B, 2 * D), jnp.bfloat16),
        in_specs=[any_spec] * 10,
        out_specs=pl.BlockSpec(memory_space=pltpu.VMEM),
        scratch_shapes=[
            pltpu.VMEM((2, B, D), jnp.bfloat16),
            pltpu.VMEM((2, L, 2, W, Dh), jnp.bfloat16),
            pltpu.VMEM((2, 2, D, HD), jnp.bfloat16),
            pltpu.VMEM((2, 8, D), jnp.float32),
            pltpu.VMEM((L, 2, R, Dh), jnp.bfloat16),
            pltpu.VMEM((L, 2, R, W), jnp.bfloat16),
            pltpu.VMEM((L, 2, R, Dh), jnp.float32),
            pltpu.VMEM((L, 2, R, Dh), jnp.float32),
            pltpu.VMEM((R, Dh), jnp.float32),
            pltpu.SemaphoreType.DMA((2,)),
            pltpu.SemaphoreType.DMA((2, L, 2)),
            pltpu.SemaphoreType.DMA((2, 2)),
            pltpu.SemaphoreType.DMA((1,)),
        ],
        compiler_params=pltpu.CompilerParams(
            vmem_limit_bytes=100 * 1024 * 1024,
            disable_bounds_checks=True,
            disable_semaphore_checks=True,
        ),
    )(A_x.reshape(B, D), A_k_cache, A_v_cache, A_wq, A_wo.T,
      B_x.reshape(B, D), B_k_cache, B_v_cache, B_wq, B_wo.T)
    return out.reshape(B, Sq, 2 * D)
```

```python
import functools

import jax
import jax.numpy as jnp
from jax import lax
import jax.experimental.pallas as pl
import jax.experimental.pallas.tpu as pltpu

_NT = (((1,), (1,)), ((), ()))
_NN = (((1,), (0,)), ((), ()))

_L = 4
_CR = 128
_LAG = 30
_VLAG = 64
_QPOS = 12
_OPOS = 76
_WPARTS = 4
_WLATE = 4
_WPRE = 2
_MV = 4
_OFFS = (-8, 16)
_SLAB = (((0, 256), (512, 64)), ((256, 256),))


@jax.jit
def pallas_concat_heads__sliding_block_cached__sliding_block_cached__decode_kernel(
    A_x: jax.Array,
    A_k_cache: jax.Array,
    A_v_cache: jax.Array,
    A_wq: jax.Array,
    A_wo: jax.Array,
    B_x: jax.Array,
    B_k_cache: jax.Array,
    B_v_cache: jax.Array,
    B_wq: jax.Array,
    B_wo: jax.Array,
):
    B, Sq, D = A_x.shape
    Hq, Dh = 32, 128
    Hkv, Sk = A_k_cache.shape[1], A_k_cache.shape[2]
    W = min(4096, max(256, Sk // 4))
    rep = Hq // Hkv
    L, CR = _L, _CR
    S0 = Sk - W
    C = rep * Dh
    HD = Hq * Dh
    R = 8 * rep
    scale = Dh ** -0.5
    NCH = W // CR
    LP = L // 2
    N = (2 * B * Hkv) // L
    NHG = N // B
    ST = NCH // L
    SLOT = ST * 2 * L
    RBP = (D // 8) // _WPARTS
    WH = HD // 2
    assert (B, Sq, rep, NCH, L) == (4, 1, 2, 16, 4) and D == 8 * _WPARTS * RBP
    assert _LAG < SLOT and _LAG % 2 == 0 and _VLAG == 2 * SLOT and NHG * LP == Hkv
    assert _WLATE * _WPARTS * 4 == L * NCH
    assert sum(nn for grp in _SLAB for _, nn in grp) == D

    def lane_prob(j):
        return 1 - j // LP

    def head_of(hg, j):
        return hg + (j % LP) * NHG

    def rows_of(j, c):
        off = _OFFS[lane_prob(j)]
        lo = 0 if c == 0 else c * CR + off
        hi = W if c == NCH - 1 else (c + 1) * CR + off
        return lo, hi - lo

    def unit_info(n):
        return n % B, n // B, n % 2

    PZ = lane_prob(L - 1)
    HZ = head_of(NHG - 1, L - 1)
    assert (HZ + 1) * C == HD
    slab_rows = [[(r0, 64) for n0, nn in grp for r0 in range(n0, n0 + nn, 64)] for grp in _SLAB]

    s0, s1 = [], []
    for s in range(ST * (L - 1)):
        for j in range(L):
            if s < ST * j:
                s1.append((1, j, N - 2, *rows_of(j, s)))
                s0.append((0, j, N - 1, *rows_of(j, s)))

    def v_last(j, cs):
        return [(1, j, N - 1, *rows_of(j, c)) for c in cs]

    half = NCH // 2
    s0 += v_last(0, range(half))
    s0 += [e for pair in zip(v_last(0, range(half, NCH)), v_last(1, range(half, NCH))) for e in pair]
    s0 += v_last(1, range(half)) + v_last(2, range(_MV))
    s1 += v_last(2, range(_MV, NCH)) + v_last(3, range(NCH))
    s1 += [(2, grp, 0, r0, nr) for grp in range(2) for r0, nr in slab_rows[grp]]
    ready = {(1, 2, N - 3): _LAG, (1, 3, N - 3): _LAG + SLOT}
    for j in range(L):
        ready[(0, j, N - 1)] = _LAG
        ready[(1, j, N - 2)] = _LAG + _VLAG
    for lst, lag in ((s0, _LAG), (s1, _LAG + _VLAG)):
        for x, e in enumerate(lst):
            ready[e[:3]] = max(ready.get(e[:3], 0), 2 * (x + 1) + lag)
            assert ready.get((e[0], e[1], e[2] - 2), 0) <= 2 * x
    for j in range(L):
        assert ready[(0, j, N - 1)] < ready[(1, j, N - 1)] and ready[(1, j, N - 2)] < ready[(1, j, N - 1)]
        assert ready.get((1, j, N - 3), 0) <= ready[(0, j, N - 1)]
    assert ready[(1, 0, N - 1)] < ready[(1, 1, N - 1)]
    assert ready[(1, 2, N - 1)] < ready[(1, 3, N - 1)] < ready[(2, 0, 0)] < ready[(2, 1, 0)]

    def kernel(xa, ka, va, wqa, woa, xb, kb, vb, wqb, wob, o_ref,
               xbuf, kvbuf, wbuf, acc_ref, q_ref, p_ref, l_ref, oh_ref,
               xsem, kvsem, wsem, zsem):
        probs = ((xa, ka, va, wqa, woa), (xb, kb, vb, wqb, wob))

        def kv_start(info, j, kv, r0, nr, prio):
            b, hg, slot = info
            pltpu.make_async_copy(
                probs[lane_prob(j)][1 + kv].at[b, head_of(hg, j), pl.ds(S0 + r0, nr), :],
                kvbuf.at[kv, j, slot, pl.ds(r0, nr), :],
                kvsem.at[kv, j, slot],
            ).start(priority=prio)

        def wait_block(kv, j, slot):
            pltpu.make_async_copy(kvbuf.at[kv, j, slot], kvbuf.at[kv, j, slot], kvsem.at[kv, j, slot]).wait()

        def w_cols(p, w):
            return HD - C if (p, w) == (PZ, 1) else HD

        def w_start(p, w, r, part, hf, prio):
            r0 = (part * RBP + r) * 8
            if not isinstance(r0, int):
                r0 = pl.multiple_of(r0, 8)
            cs = pl.ds(hf * WH, min(WH, w_cols(p, w) - hf * WH))
            pltpu.make_async_copy(
                probs[p][3 + w].at[pl.ds(r0, 8), cs], wbuf.at[p, w, pl.ds(r0, 8), cs], wsem.at[p, w],
            ).start(priority=prio)

        def wait_weight(p, w):
            v = wbuf.at[p, w, :, pl.ds(0, w_cols(p, w))]
            pltpu.make_async_copy(v, v, wsem.at[p, w]).wait()

        def slab_copy(grp, r0, nr):
            return pltpu.make_async_copy(
                probs[PZ][4].at[pl.ds(r0, nr), pl.ds(HZ * C, C)],
                wbuf.at[PZ, 1, pl.ds(r0, nr), pl.ds(HZ * C, C)],
                zsem.at[grp],
            )

        x_copies = [pltpu.make_async_copy(probs[p][0], xbuf.at[p], xsem.at[p]) for p in range(2)]

        def weight_rows(w, r, carry):
            for hf in range(2):
                for part in range(_WPARTS):
                    for p in (1, 0):
                        w_start(p, w, r, part, hf, p)
            return carry

        n_mid = RBP - _WLATE - _WPRE
        for r in range(n_mid, n_mid + _WPRE):
            for hf in range(2):
                for p in (1, 0):
                    for part in range(_WPARTS):
                        w_start(p, 1, r, part, hf, 1)
        lax.fori_loop(0, RBP, functools.partial(weight_rows, 0), 0)
        for p in range(2):
            x_copies[p].start()
        lax.fori_loop(0, n_mid, functools.partial(weight_rows, 1), 0)
        late_w = [(p, 1, r, part, hf) for p in (1, 0) for r in range(RBP - _WLATE, RBP)
                  for hf in range(2) for part in range(_WPARTS)]

        row_b = lax.broadcasted_iota(jnp.int32, (R, Dh), 0) % B
        acc_ref[...] = jnp.zeros_like(acc_ref)
        oh_ref[...] = jnp.zeros_like(oh_ref)

        def cols(h):
            return pl.ds(h * C if isinstance(h, int) else pl.multiple_of(h * C, C), C)

        def qproj(j, hg, par):
            p = lane_prob(j)
            x4 = xbuf[p].astype(jnp.float32)
            x8 = jnp.concatenate([x4, x4], axis=0).astype(jnp.bfloat16)
            qf = lax.dot_general(x8, wbuf[p, 0, :, cols(head_of(hg, j))], _NN,
                                 preferred_element_type=jnp.float32)
            q_ref[j, par] = jnp.concatenate([qf[:, :Dh], qf[:, Dh:]], axis=0).astype(jnp.bfloat16)

        def scores_softmax(j, info):
            _, hg, slot = info
            s = lax.dot_general(q_ref[j, hg % 2], kvbuf[0, j, slot], _NT,
                                preferred_element_type=jnp.float32) * scale
            m = jnp.max(s, axis=-1, keepdims=True)
            e = jnp.exp(s - m)
            l_ref[j, slot] = jnp.broadcast_to(jnp.sum(e, axis=-1, keepdims=True), (R, Dh))
            p_ref[j, slot] = e.astype(jnp.bfloat16)

        def pv(j, info):
            b, hg, slot = info
            o = lax.dot_general(p_ref[j, slot], kvbuf[1, j, slot], _NN,
                                preferred_element_type=jnp.float32)
            oh_ref[j, hg % 2] = jnp.where(row_b == b, o / l_ref[j, slot], oh_ref[j, hg % 2])

        def head_out(j, hg, valid=None):
            o = oh_ref[j, hg % 2]
            if valid is not None:
                o = jnp.where(valid, o, 0.0)
            return jnp.concatenate([o[0:8], o[8:16]], axis=1).astype(jnp.bfloat16)

        def oproj(j, hg, valid=None):
            p = lane_prob(j)
            acc_ref[p] += lax.dot_general(head_out(j, hg, valid), wbuf[p, 1, :, cols(head_of(hg, j))], _NT,
                                          preferred_element_type=jnp.float32)

        def iteration(i):
            static = isinstance(i, int)
            infos = {d: unit_info(i - d) if (not static or i - d >= 0) else None for d in range(4)}
            actions = {}

            def consume(t):
                ik = infos[1]
                jv = (t - 2) % L
                iv = infos[2 if t >= 2 else 3]
                if ik is not None:
                    wait_block(0, t, ik[2])
                if iv is not None:
                    wait_block(1, jv, iv[2])
                if ik is not None:
                    scores_softmax(t, ik)
                if iv is not None:
                    pv(jv, iv)

            for t in range(L):
                actions[SLOT * t + _LAG] = functools.partial(consume, t)
            hgq = (i - 1) // L + 1
            if static:
                if i >= 1:
                    actions[_QPOS] = functools.partial(qproj, (i - 1) % L, hgq, hgq % 2)
            else:
                actions[_QPOS] = functools.partial(qproj, (i - 1) % L, jnp.minimum(hgq, NHG - 1), hgq % 2)
                io = jnp.maximum(i - 6, 0)
                actions[_OPOS] = functools.partial(oproj, io % L, io // L, i >= 6)
            idx = 0
            for s in range(NCH):
                for j in range(L):
                    dk = 0 if s >= ST * j else 1
                    ik, iv = infos[dk], infos[dk + 1]
                    if idx in actions:
                        actions[idx]()
                    if iv is not None:
                        kv_start(iv, j, 1, *rows_of(j, s), 1)
                    elif ik is not None:
                        w_start(*late_w.pop(0), 1)
                    if ik is not None:
                        kv_start(ik, j, 0, *rows_of(j, s), 0)
                    idx += 2

        iteration(0)
        for p in range(2):
            x_copies[p].wait()
            wait_weight(p, 0)
        for j in range(L):
            qproj(j, 0, 0)
        iteration(1)
        assert not late_w
        iteration(2)
        for p in range(2):
            wait_weight(p, 1)

        def body(i, carry):
            iteration(i)
            return carry

        lax.fori_loop(3, N, body, 0)

        def end_k(j, n):
            info = unit_info(n)
            wait_block(0, j, info[2])
            scores_softmax(j, info)

        def end_v(j, n):
            info = unit_info(n)
            wait_block(1, j, info[2])
            pv(j, info)
            if n == N - 1 and j != L - 1:
                oproj(j, NHG - 1)
                if j == LP - 1:
                    p = lane_prob(j)
                    o_ref[:, p * D:(p + 1) * D] = acc_ref[p, 0:B, :].astype(o_ref.dtype)

        def end_slab(grp, _):
            for r0, nr in slab_rows[grp]:
                slab_copy(grp, r0, nr).wait()
            z = head_out(L - 1, NHG - 1)
            for n0, nn in _SLAB[grp]:
                y = acc_ref[PZ, :, pl.ds(n0, nn)] + lax.dot_general(
                    z, wbuf[PZ, 1, pl.ds(n0, nn), pl.ds(HZ * C, C)], _NT, preferred_element_type=jnp.float32)
                o_ref[:, pl.ds(PZ * D + n0, nn)] = y[0:B].astype(o_ref.dtype)

        events = [(pos, -kind, functools.partial((end_k, end_v, end_slab)[kind], j, n))
                  for (kind, j, n), pos in ready.items()]
        events.append((4, 0, functools.partial(oproj, 2, NHG - 2)))
        events.append((16, 0, functools.partial(oproj, 3, NHG - 2)))
        events.sort(key=lambda e: e[:2])
        for x in range(max(len(s0), len(s1))):
            while events and events[0][0] <= 2 * x:
                events.pop(0)[2]()
            for prio, lst in ((1, s1), (0, s0)):
                if x < len(lst):
                    kind, j, n, r0, nr = lst[x]
                    if kind == 2:
                        slab_copy(j, r0, nr).start(priority=prio)
                    else:
                        kv_start(unit_info(n), j, kind, r0, nr, prio)
        for e in events:
            e[2]()

    any_spec = pl.BlockSpec(memory_space=pl.ANY)
    out = pl.pallas_call(
        kernel,
        out_shape=jax.ShapeDtypeStruct((B, 2 * D), jnp.bfloat16),
        in_specs=[any_spec] * 10,
        out_specs=pl.BlockSpec(memory_space=pltpu.VMEM),
        scratch_shapes=[
            pltpu.VMEM((2, B, D), jnp.bfloat16),
            pltpu.VMEM((2, L, 2, W, Dh), jnp.bfloat16),
            pltpu.VMEM((2, 2, D, HD), jnp.bfloat16),
            pltpu.VMEM((2, 8, D), jnp.float32),
            pltpu.VMEM((L, 2, R, Dh), jnp.bfloat16),
            pltpu.VMEM((L, 2, R, W), jnp.bfloat16),
            pltpu.VMEM((L, 2, R, Dh), jnp.float32),
            pltpu.VMEM((L, 2, R, Dh), jnp.float32),
            pltpu.SemaphoreType.DMA((2,)),
            pltpu.SemaphoreType.DMA((2, L, 2)),
            pltpu.SemaphoreType.DMA((2, 2)),
            pltpu.SemaphoreType.DMA((2,)),
        ],
        compiler_params=pltpu.CompilerParams(
            vmem_limit_bytes=64 * 1024 * 1024,
            disable_bounds_checks=True,
            disable_semaphore_checks=True,
        ),
    )(A_x.reshape(B, D), A_k_cache, A_v_cache, A_wq, A_wo.T,
      B_x.reshape(B, D), B_k_cache, B_v_cache, B_wq, B_wo.T)
    return out.reshape(B, Sq, 2 * D)
```
